```python
import os as _os
_os.environ.setdefault("JAX_PLATFORMS", "cpu")
import jax
import jax.numpy as jnp

def _softmax(x, axis=-1):
    return jax.nn.softmax(x, axis=axis)
def _gelu(x):
    return jax.nn.gelu(x, approximate=True)
def _silu(x):
    return jax.nn.silu(x)
def _sigmoid(x):
    return jax.nn.sigmoid(x)
def _layernorm(x, axis=-1, eps=1e-5):
    m = jnp.mean(x, axis=axis, keepdims=True)
    v = jnp.var(x, axis=axis, keepdims=True)
    return (x - m) / jnp.sqrt(v + eps)
def _scatter_add(tgt, idx, src, axis=0):
    return tgt.at[idx].add(src)
def _segment_sum(src, seg, n):
    return jax.ops.segment_sum(src, seg, n)
class _Rng:
    def __init__(self, key):
        self._k = key
    def _next(self):
        self._k, sub = jax.random.split(self._k)
        return sub
    def normal(self, shape):
        return jax.random.normal(self._next(), shape, dtype=jnp.bfloat16)
    def randint(self, lo, hi, shape):
        return jax.random.randint(self._next(), shape, lo, hi, dtype=jnp.int32)
    def uniform(self, shape, lo=0.0, hi=1.0):
        return jax.random.uniform(self._next(), shape, jnp.bfloat16, lo, hi)
    def permutation(self, n):
        return jax.random.permutation(self._next(), n)


kernel_name = 'sequential_preLN__mha_block__mixer_token_mlp__prompt'

def setup_inputs():
    _rng = _Rng(jax.random.key(int.from_bytes(__import__("os").urandom(4), "little")))
    _w = (lambda a: (lambda t: t.astype(jnp.bfloat16) if jnp.issubdtype(t.dtype, jnp.floating) else t)(jnp.asarray(a)))
    def _A_setup():
        B, S, D, H = 1, 2048, 448, 16
        return {
            "x": _w((lambda *s: _rng.normal(s) * 0.05)(B, S, D)),
            "wqkv": _w((lambda *s: _rng.normal(s) * 0.05)(D, 3 * D)),
            "wo": _w((lambda *s: _rng.normal(s) * 0.05)(D, D)),
        }
    _A_in = _A_setup()

    def _B_setup():
        B, S, D, F = 1, 2048, 448, 1792
        return {
            "x": _w((lambda *s: _rng.normal(s) * 0.05)(B, S, D)),
            "w1": _w((lambda *s: _rng.normal(s) * 0.2)(S, F) * (S ** -0.5)),
            "b1": _w((lambda *s: _rng.normal(s) * 0.2)(F) * 0.02),
            "w2": _w((lambda *s: _rng.normal(s) * 0.2)(F, S) * (F ** -0.5)),
            "b2": _w((lambda *s: _rng.normal(s) * 0.05)(S) * 0.02),
        }
    _B_in = _B_setup()

    return {
        "A_x": _A_in["x"],
        "A_wqkv": _A_in["wqkv"],
        "A_wo": _A_in["wo"],
        "B_x": _B_in["x"],
        "B_w1": _B_in["w1"],
        "B_b1": _B_in["b1"],
        "B_w2": _B_in["w2"],
        "B_b2": _B_in["b2"],
    }

def reference(A_x, A_wqkv, A_wo, B_x, B_w1, B_b1, B_w2, B_b2):
    def _A_ref(x, wqkv, wo):
        B, S, D = x.shape
        H = 16
        Dh = D // H
        qkv = (lambda x, *d: x.transpose(*d))((x @ wqkv).reshape(B, S, 3, H, Dh), 2, 0, 3, 1, 4)
        q, k, v = qkv[0], qkv[1], qkv[2]
        scores = jnp.einsum("bhqd,bhkd->bhqk", q, k) * (Dh ** -0.5)
        p = _softmax(scores, axis=-1)
        o = jnp.einsum("bhqk,bhkd->bhqd", p, v)
        return (lambda x, *d: x.transpose(*d))(o, 0, 2, 1, 3).reshape(B, S, D) @ wo

    def _B_ref(x, w1, b1, w2, b2):
        B, S, D = x.shape
        h = _layernorm(x, axis=-1)
        u = jnp.einsum("bsd,sf->bdf", h, w1) + b1
        u = _gelu(u)
        y = jnp.einsum("bdf,fs->bds", u, w2) + b2
        return (lambda x, *d: x.transpose(*d))(y, 0, 2, 1)

    x = A_x
    h = x + _A_ref(_layernorm(x, axis=-1), A_wqkv, A_wo)
    h2 = h + _B_ref(_layernorm(h, axis=-1), B_w1, B_b1, B_w2, B_b2)
    return h2
```

```python
import jax
import jax.numpy as jnp
import jax.experimental.pallas as pl
import jax.experimental.pallas.tpu as pltpu

S, D, H, F = 2048, 448, 16, 1792
DH = D // H
HP = 32
DP = H * HP
BQ = 512
KC = 256
FC = 256
NQ = S // BQ
NK = S // KC
EPS = 1e-5
LOG2E = 1.4426950408889634
F32, BF16 = jnp.float32, jnp.bfloat16


def _dot(a, b):
    return jnp.dot(a, b, preferred_element_type=F32)


def _ln_t(xt):
    m = jnp.sum(xt, axis=0, keepdims=True) * (1.0 / D)
    c = xt - m
    v = jnp.sum(c * c, axis=0, keepdims=True) * (1.0 / D)
    return c * jax.lax.rsqrt(v + EPS)


def _kernel(x_ref, wqkv_ref, wo_ref, w1_hbm, b1_ref, w2_hbm, b2_ref, o_hbm,
            w1_ref, w2_ref, pad_ref, wt_ref, wtp_ref, wot_ref, ht_ref, ln_ref,
            q_ref, k_ref, v_ref, sa_ref, sb_ref, ot_ref, g_ref, ob_ref, sems, osems):
    cp1 = pltpu.make_async_copy(w1_hbm, w1_ref, sems.at[0])
    cp2 = pltpu.make_async_copy(w2_hbm, w2_ref, sems.at[1])
    cp1.start()
    cp2.start()

    wt_ref[:, D:] = jnp.zeros((3 * D + 64, 512 - D), F32)
    for c in range(11):
        w = min(128, 3 * D - 128 * c)
        blk = wqkv_ref[:, 128 * c:128 * c + w].astype(F32)
        if w < 128:
            blk = jnp.concatenate([blk, jnp.zeros((D, 128 - w), F32)], axis=1)
        wt_ref[128 * c:128 * (c + 1), :D] = blk.T
    zero4 = jnp.zeros((HP - DH, 512), F32)
    for h in range(3 * H):
        blk = jnp.concatenate([wt_ref[DH * h:DH * (h + 1), :], zero4], axis=0)
        wtp_ref[HP * h:HP * (h + 1), :] = blk.astype(BF16)
    for h in range(H):
        pad_ref[HP * h:HP * (h + 1), :D] = jnp.concatenate(
            [wo_ref[DH * h:DH * (h + 1), :].astype(F32), jnp.zeros((HP - DH, D), F32)], axis=0)
    pad_ref[:, D:] = jnp.zeros((DP, 512 - D), F32)
    wot_ref[...] = pad_ref[...].T[:D].astype(BF16)

    row = jax.lax.broadcasted_iota(jnp.int32, (DP, BQ), 0)
    ones_row = (row & (HP - 1)) == DH
    ln_ref[D:, :] = jnp.zeros((512 - D, S), BF16)
    for t in range(NQ):
        ts = slice(t * BQ, (t + 1) * BQ)
        xb = jnp.concatenate([x_ref[ts, :].astype(F32), jnp.zeros((BQ, 512 - D), F32)], axis=1)
        xt = xb.T[:D]
        ht_ref[t] = xt
        ln_ref[:D, ts] = _ln_t(xt).astype(BF16)
        ln = ln_ref[:, ts]
        qt = _dot(wtp_ref[0:DP, :], ln) * (DH ** -0.5 * LOG2E)
        q_ref[t] = qt.astype(BF16)
        kt = _dot(wtp_ref[DP:2 * DP, :], ln)
        kk = kt.T.astype(BF16)
        for g in range(4):
            k_ref[g, ts, :] = kk[:, 128 * g:128 * (g + 1)]
        vt = _dot(wtp_ref[2 * DP:3 * DP, :], ln)
        v_ref[:, ts] = jnp.where(ones_row, 1.0, vt).astype(BF16)

    qrow = jax.lax.broadcasted_iota(jnp.int32, (128, BQ), 0) // HP

    def load_q(i):
        h = i // NQ
        g = h // 4
        q = q_ref[i % NQ, pl.ds(pl.multiple_of(g * 128, 128), 128), :]
        return g, jnp.where(qrow == h % 4, q, jnp.zeros_like(q))

    def qk_chunk(g, q, s_ref, c, m):
        s = _dot(k_ref[g, c * KC:(c + 1) * KC, :], q)
        s_ref[c * KC:(c + 1) * KC, :] = s
        mc = jnp.max(s.reshape(KC // 8, 8, BQ), axis=0)
        return mc if m is None else jnp.maximum(m, mc)

    def step(i, m, src, dst):
        g, q = load_q(jnp.minimum(i + 1, H * NQ - 1))
        hrow = pl.ds(pl.multiple_of((i // NQ) * HP, HP), HP)
        mn = acc = None
        for c in range(NK):
            mn = qk_chunk(g, q, dst, c, mn)
            p = jnp.exp2(src[c * KC:(c + 1) * KC, :] - m).astype(BF16)
            o = _dot(v_ref[hrow, c * KC:(c + 1) * KC], p)
            acc = o if acc is None else acc + o
        ot_ref[i % NQ, hrow, :] = (acc * (1.0 / acc[DH:DH + 1, :])).astype(BF16)
        return jnp.max(mn, axis=0, keepdims=True)

    g0, q0 = load_q(0)
    m0 = None
    for c in range(NK):
        m0 = qk_chunk(g0, q0, sa_ref, c, m0)
    m0 = jnp.max(m0, axis=0, keepdims=True)

    def body(j, m):
        m = step(2 * j, m, sa_ref, sb_ref)
        return step(2 * j + 1, m, sb_ref, sa_ref)

    jax.lax.fori_loop(0, H * NQ // 2, body, m0)

    for t in range(NQ):
        ht = ht_ref[t] + _dot(wot_ref[...], ot_ref[t])
        ht_ref[t] = ht
        ln_ref[:D, t * BQ:(t + 1) * BQ] = _ln_t(ht).astype(BF16)

    cp1.wait()
    for f in range(F // FC):
        fs = slice(f * FC, (f + 1) * FC)
        u = _dot(ln_ref[:D, :], w1_ref[:, fs]) + b1_ref[:, fs]
        g_ref[:, fs] = jax.nn.gelu(u, approximate=True).astype(BF16)
    cp2.wait()
    outs = []
    for t in range(NQ):
        ts = slice(t * BQ, (t + 1) * BQ)
        y = ht_ref[t] + _dot(g_ref[...], w2_ref[:, ts]) + b2_ref[:, ts]
        yt = jnp.concatenate([y, jnp.zeros((512 - D, BQ), F32)], axis=0).T
        ob_ref[ts, :] = yt[:, :D].astype(BF16)
        cp = pltpu.make_async_copy(ob_ref.at[ts, :], o_hbm.at[ts, :], osems.at[t])
        cp.start()
        outs.append(cp)
    for cp in outs:
        cp.wait()


@jax.jit
def pallas_sequential_preLN__mha_block__mixer_token_mlp__prompt_kernel(
    A_x: jax.Array,
    A_wqkv: jax.Array,
    A_wo: jax.Array,
    B_x: jax.Array,
    B_w1: jax.Array,
    B_b1: jax.Array,
    B_w2: jax.Array,
    B_b2: jax.Array,
):
    del B_x
    vmem = pl.BlockSpec(memory_space=pltpu.VMEM)
    hbm = pl.BlockSpec(memory_space=pl.ANY)
    out = pl.pallas_call(
        _kernel,
        in_specs=[vmem, vmem, vmem, hbm, vmem, hbm, vmem],
        out_specs=hbm,
        out_shape=jax.ShapeDtypeStruct((S, D), BF16),
        scratch_shapes=[
            pltpu.VMEM((S, F), BF16),
            pltpu.VMEM((F, S), BF16),
            pltpu.VMEM((DP, 512), F32),
            pltpu.VMEM((3 * D + 64, 512), F32),
            pltpu.VMEM((3 * DP, 512), BF16),
            pltpu.VMEM((D, DP), BF16),
            pltpu.VMEM((NQ, D, BQ), F32),
            pltpu.VMEM((512, S), BF16),
            pltpu.VMEM((NQ, DP, BQ), BF16),
            pltpu.VMEM((4, S, 128), BF16),
            pltpu.VMEM((DP, S), BF16),
            pltpu.VMEM((S, BQ), F32),
            pltpu.VMEM((S, BQ), F32),
            pltpu.VMEM((NQ, DP, BQ), BF16),
            pltpu.VMEM((D, F), BF16),
            pltpu.VMEM((S, D), BF16),
            pltpu.SemaphoreType.DMA((2,)),
            pltpu.SemaphoreType.DMA((NQ,)),
        ],
        compiler_params=pltpu.CompilerParams(vmem_limit_bytes=100 * 1024 * 1024),
    )(A_x.reshape(S, D), A_wqkv, A_wo, B_w1, B_b1.reshape(1, F), B_w2, B_b2.reshape(1, S))
    return out.reshape(1, S, D)
```

```python
import jax
import jax.numpy as jnp
import jax.experimental.pallas as pl
import jax.experimental.pallas.tpu as pltpu

S, D, H, F = 2048, 448, 16, 1792
DH = D // H
HP = 32
DP = H * HP
GR = 4 * DH
BQ = 1024
KC = 128
TB = 512
FC = 256
OC = 256
NQ = S // BQ
NIT = H * NQ
EPS = 1e-5
LOG2E = 1.4426950408889634
F32, BF16 = jnp.float32, jnp.bfloat16


def _dot(a, b):
    return jnp.dot(a, b, preferred_element_type=F32)


def _ln_t(xt):
    m = jnp.sum(xt, axis=0, keepdims=True) * (1.0 / D)
    c = xt - m
    v = jnp.sum(c * c, axis=0, keepdims=True) * (1.0 / D)
    return c * jax.lax.rsqrt(v + EPS)


def _window(h):
    off = (DH * h) % 8
    return DH * h - off, off


def _qrows(j):
    return j * DH // 16 * 16, -(-(j + 1) * DH // 16) * 16


def _kernel(x_hbm, wqkv_hbm, wo_hbm, w1_hbm, b1_in, w2_hbm, b2_in, o_hbm, b1_ref, b2_ref,
            x_ref, wqkv_ref, wo_ref, w1_ref, w2_ref, wt_ref, wot_ref, ht_ref, ln_ref,
            q_ref, k_ref, v_ref, s_ref, ot_ref, g_ref, ob_ref, sems, xsems, osems):
    cp_wk, *cp_wrest = [
        pltpu.make_async_copy(wqkv_hbm.at[:, ws], wqkv_ref.at[:, ws], sems.at[3 + n])
        for n, ws in enumerate([slice(384, 896), slice(0, 384), slice(896, 3 * D)])]
    cp_wo = pltpu.make_async_copy(wo_hbm, wo_ref, sems.at[0])
    cp_w1 = pltpu.make_async_copy(w1_hbm, w1_ref, sems.at[1])
    cp_w2 = pltpu.make_async_copy(w2_hbm, w2_ref, sems.at[2])
    tsl = [slice(t * TB, (t + 1) * TB) for t in range(S // TB)]

    cp_x = [pltpu.make_async_copy(x_hbm.at[:, ts], x_ref.at[:, ts], xsems.at[t])
            for t, ts in enumerate(tsl)]
    cp_x[0].start()
    cp_wk.start()

    ln_ref[D:, :] = jnp.zeros((512 - D, S), BF16)

    @pl.loop(0, 4)
    def _(g):
        for j in range(4):
            lo, hi = _qrows(j)
            if lo > 0:
                q_ref[4 * g + j, :lo, :] = jnp.zeros((lo, S), BF16)
            if hi < 128:
                q_ref[4 * g + j, hi:, :] = jnp.zeros((128 - hi, S), BF16)

    def transpose_w(cols, blk):
        wt_ref[cols, :] = jnp.concatenate([blk, jnp.zeros((512 - D, 128), BF16)], axis=0).T

    def transpose_tiles(tiles):
        for c in tiles:
            w = min(128, 3 * D - 128 * c)
            transpose_w(slice(128 * c, 128 * (c + 1)),
                        wqkv_ref[:, 128 * c:128 * c + w] if w == 128 else jnp.concatenate(
                            [wqkv_ref[:, 128 * c:], jnp.zeros((D, 128 - w), BF16)], axis=1))

    def ln1(ts):
        ln_ref[:D, ts] = _ln_t(x_ref[:, ts].astype(F32)).astype(BF16)

    vrow = jax.lax.broadcasted_iota(jnp.int32, (HP, TB), 0)
    qrow = jax.lax.broadcasted_iota(jnp.int32, (128, TB), 0)
    pad = jnp.zeros((128 - GR, TB), F32)

    def project_k(ts):
        kt = _dot(wt_ref[D:2 * D, :], ln_ref[:, ts]).astype(BF16)
        for g in range(4):
            k_ref[g, ts, :] = jnp.concatenate(
                [kt[GR * g:GR * (g + 1)], jnp.zeros((128 - GR, TB), BF16)], axis=0).T

    cp_x[0].wait()
    cp_x[1].start()
    ln1(tsl[0])
    cp_wk.wait()
    for cp in cp_wrest + cp_x[2:] + [cp_wo]:
        cp.start()
    transpose_tiles(range(3, 7))
    cp_x[1].wait()
    ln1(tsl[1])
    project_k(tsl[0])
    for cp in cp_wrest + cp_x[2:]:
        cp.wait()
    rest = [0, 1, 2, 7, 8, 9, 10]
    nt = len(tsl) - 1
    for t in range(1, len(tsl)):
        if t + 1 < len(tsl):
            ln1(tsl[t + 1])
        project_k(tsl[t])
        transpose_tiles(rest[(t - 1) * len(rest) // nt:t * len(rest) // nt])

    def project_vq(t, _):
        ts = pl.ds(pl.multiple_of(t * TB, TB), TB)
        vt = _dot(wt_ref[2 * D:3 * D, :], ln_ref[:, ts])
        for h in range(H):
            r0, off = _window(h)
            v_ref[h, :, ts] = jnp.where(vrow == (DH if off == 0 else 0), 1.0, vt[r0:r0 + HP]).astype(BF16)
        qt = jnp.concatenate([_dot(wt_ref[:D, :], ln_ref[:, ts]) * (DH ** -0.5 * LOG2E), pad], axis=0)
        for h in range(H):
            g, j = divmod(h, 4)
            lo, hi = _qrows(j)
            keep = (qrow >= j * DH) & (qrow < (j + 1) * DH)
            q_ref[h, lo:hi, ts] = jnp.where(keep, qt[GR * g:GR * g + 128], 0.0)[lo:hi].astype(BF16)

    jax.lax.fori_loop(0, S // TB, project_vq, None, unroll=1)

    nch = S // KC

    def qcols(i):
        return pl.ds(pl.multiple_of((i % NQ) * BQ, BQ), BQ)

    def chunks(odd):
        return range(nch - 1, -1, -1) if odd else range(nch)

    def slot(c, odd):
        lo = (c + (0 if odd else 1)) * KC
        return slice(lo, lo + KC)

    def qk_chunk(i, odd, q, c, m):
        s = _dot(k_ref[i // (4 * NQ), c * KC:(c + 1) * KC, :], q)
        s_ref[slot(c, odd), :] = s
        mc = jnp.max(s.reshape(KC // 8, 8, BQ), axis=0)
        return mc if m is None else jnp.maximum(m, mc)

    def pv_chunk(i, odd, m, c, acc):
        p = jnp.exp2(s_ref[slot(c, odd), :] - m).astype(BF16)
        o = _dot(v_ref[i // NQ, :, c * KC:(c + 1) * KC], p)
        return o if acc is None else acc + o

    def pv_finish(i, acc):
        h = i // NQ
        den = jnp.where(h % 2 == 0, acc[DH:DH + 1, :], acc[0:1, :])
        rows = pl.ds(pl.multiple_of(h * HP, HP), HP)
        ot_ref[rows, qcols(i)] = (acc * (1.0 / den)).astype(BF16)

    def step(i, odd, m):
        q = q_ref[(i + 1) // NQ, :, qcols(i + 1)]
        mn = acc = None
        for c in chunks(odd):
            mn = qk_chunk(i + 1, not odd, q, c, mn)
            acc = pv_chunk(i, odd, m, c, acc)
        pv_finish(i, acc)
        return jnp.max(mn, axis=0, keepdims=True)

    def two_steps(j, m):
        @pl.when(j == 1)
        def _():
            cp_w1.start()
            cp_w2.start()

        return step(2 * j + 1, True, step(2 * j, False, m))

    q0 = q_ref[0, :, 0:BQ]
    m0 = None
    for c in range(nch):
        m0 = qk_chunk(0, False, q0, c, m0)
    m_last = jax.lax.fori_loop(0, NIT // 2 - 1, two_steps, jnp.max(m0, axis=0, keepdims=True))
    m_last = step(NIT - 2, False, m_last)

    cp_wo.wait()
    wrow = jax.lax.broadcasted_iota(jnp.int32, (HP, 512), 0)
    wins = []
    for h in range(H):
        r0, off = _window(h)
        blk = jnp.concatenate([wo_ref[...].astype(F32)[r0:r0 + HP], jnp.zeros((HP, 512 - D), F32)], axis=1)
        wins.append(jnp.where((wrow >= off) & (wrow < off + DH), blk, 0.0))
    wot_ref[...] = jnp.concatenate(wins, axis=0).T[:D].astype(BF16)

    def out_proj(ts):
        ht = x_ref[:, ts].astype(F32) + _dot(wot_ref[...], ot_ref[:, ts])
        ht_ref[:, ts] = ht
        ln_ref[:D, ts] = _ln_t(ht).astype(BF16)

    half = BQ // 2
    pending = [slice(c, c + 256) for c in range(0, S - BQ, 256)]
    for part, count in enumerate((2, 3)):
        cols = slice(part * half, (part + 1) * half)
        todo, pending = pending[:count], pending[count:]
        acc = None
        for n, c in enumerate(chunks(True)):
            p = jnp.exp2(s_ref[slot(c, True), cols] - m_last[:, cols]).astype(BF16)
            o = _dot(v_ref[H - 1, :, c * KC:(c + 1) * KC], p)
            acc = o if acc is None else acc + o
            for ts in todo[n * count // nch:(n + 1) * count // nch]:
                out_proj(ts)
        lo = S - BQ + part * half
        den = acc[DH:DH + 1, :] if (H - 1) % 2 == 0 else acc[0:1, :]
        ot_ref[DP - HP:, lo:lo + half] = (acc * (1.0 / den)).astype(BF16)
        pending += [slice(c, c + 256) for c in range(lo, lo + half, 256)]
    for ts in pending:
        out_proj(ts)

    b1_ref[...] = b1_in[...].astype(F32).reshape(1, F)
    b2_ref[...] = b2_in[...].astype(F32).reshape(1, S)
    cp_w1.wait()
    cp_w2.wait()

    def hidden(f, _):
        fs = pl.ds(pl.multiple_of(f * FC, FC), FC)
        u = _dot(ln_ref[:D, :], w1_ref[:, fs]) + b1_ref[:, fs]
        g_ref[:, fs] = jax.nn.gelu(u, approximate=True).astype(BF16)

    jax.lax.fori_loop(0, F // FC, hidden, None, unroll=F // FC)

    def out_copy(t):
        ts = pl.ds(pl.multiple_of(t * OC, OC), OC)
        return pltpu.make_async_copy(ob_ref.at[:, ts], o_hbm.at[:, ts], osems.at[t])

    def tokens(t, _):
        ts = pl.ds(pl.multiple_of(t * OC, OC), OC)
        y = ht_ref[:, ts] + _dot(g_ref[...], w2_ref[:, ts]) + b2_ref[:, ts]
        ob_ref[:, ts] = y.astype(BF16)
        out_copy(t).start()

    jax.lax.fori_loop(0, S // OC, tokens, None, unroll=2)
    for t in range(S // OC):
        out_copy(t).wait()


@jax.jit
def pallas_sequential_preLN__mha_block__mixer_token_mlp__prompt_kernel(
    A_x: jax.Array,
    A_wqkv: jax.Array,
    A_wo: jax.Array,
    B_x: jax.Array,
    B_w1: jax.Array,
    B_b1: jax.Array,
    B_w2: jax.Array,
    B_b2: jax.Array,
):
    del B_x
    vmem = pl.BlockSpec(memory_space=pltpu.VMEM)
    hbm = pl.BlockSpec(memory_space=pltpu.HBM)
    out = pl.pallas_call(
        _kernel,
        in_specs=[hbm, hbm, hbm, hbm, vmem, hbm, vmem],
        out_specs=hbm,
        out_shape=jax.ShapeDtypeStruct((D, S), BF16),
        scratch_shapes=[
            pltpu.VMEM((1, F), F32),
            pltpu.VMEM((1, S), F32),
            pltpu.VMEM((D, S), BF16),
            pltpu.VMEM((D, 3 * D), BF16),
            pltpu.VMEM((D, D), BF16),
            pltpu.VMEM((S, F), BF16),
            pltpu.VMEM((F, S), BF16),
            pltpu.VMEM((3 * D + 64, 512), BF16),
            pltpu.VMEM((D, DP), BF16),
            pltpu.VMEM((D, S), F32),
            pltpu.VMEM((512, S), BF16),
            pltpu.VMEM((H, 128, S), BF16),
            pltpu.VMEM((4, S, 128), BF16),
            pltpu.VMEM((H, HP, S), BF16),
            pltpu.VMEM((S + KC, BQ), F32),
            pltpu.VMEM((DP, S), BF16),
            pltpu.VMEM((D, F), BF16),
            pltpu.VMEM((D, S), BF16),
            pltpu.SemaphoreType.DMA((6,)),
            pltpu.SemaphoreType.DMA((S // TB,)),
            pltpu.SemaphoreType.DMA((S // OC,)),
        ],
        compiler_params=pltpu.CompilerParams(
            vmem_limit_bytes=100 * 1024 * 1024,
            flags={"XLA_TPU_EVENLY_DISTRIBUTE_CRITICAL_NODES": True},
        ),
    )(A_x.reshape(S, D).T, A_wqkv, A_wo, B_w1, B_b1, B_w2, B_b2)
    return out.T.reshape(1, S, D)
```
